```python
import os as _os
_os.environ.setdefault('JAX_PLATFORMS', 'cpu')
import jax
import jax.numpy as jnp

def _softmax(x, axis=-1):
    return jax.nn.softmax(x, axis=axis)

def _gelu(x):
    return jax.nn.gelu(x, approximate=True)

def _silu(x):
    return jax.nn.silu(x)

def _sigmoid(x):
    return jax.nn.sigmoid(x)

def _layernorm(x, axis=-1, eps=1e-05):
    m = jnp.mean(x, axis=axis, keepdims=True)
    v = jnp.var(x, axis=axis, keepdims=True)
    return (x - m) / jnp.sqrt(v + eps)

def _scatter_add(tgt, idx, src, axis=0):
    return tgt.at[idx].add(src)

def _segment_sum(src, seg, n):
    return jax.ops.segment_sum(src, seg, n)

class _Rng:

    def __init__(self, key):
        self._k = key

    def _next(self):
        self._k, sub = jax.random.split(self._k)
        return sub

    def normal(self, shape):
        return jax.random.normal(self._next(), shape, dtype=jnp.bfloat16)

    def randint(self, lo, hi, shape):
        return jax.random.randint(self._next(), shape, lo, hi, dtype=jnp.int32)

    def uniform(self, shape, lo=0.0, hi=1.0):
        return jax.random.uniform(self._next(), shape, jnp.bfloat16, lo, hi)

    def permutation(self, n):
        return jax.random.permutation(self._next(), n)
kernel_name = 'standalone__autoregressive_conv_wavenet__speech'

def setup_inputs():
    _rng = _Rng(jax.random.key(int.from_bytes(__import__("os").urandom(4), "little")))
    _w = lambda a: (lambda t: t.astype(jnp.bfloat16) if jnp.issubdtype(t.dtype, jnp.floating) else t)(jnp.asarray(a))
    B, T, D, K = (2, 4000, 512, 31)
    return {'x': _w((lambda *s: _rng.normal(s) * 0.05)(B, T, D)), 'w': _w((lambda *s: _rng.normal(s) * 0.05)(K, D, 2 * D)), 'w_o': _w((lambda *s: _rng.normal(s) * 0.05)(D, D))}

def reference(x, w, w_o):
    B, T, D = x.shape
    K = w.shape[0]
    dil = 2
    pad = (K - 1) * dil
    xp = jnp.pad(x, ((0, 0), (pad, 0), (0, 0)))
    h = jnp.einsum('btc,cd->btd', xp[:, pad:pad + T, :], w[0])
    for i in range(1, K):
        off = pad - i * dil
        h = h + jnp.einsum('btc,cd->btd', xp[:, off:off + T, :], w[i])
    f = h[..., :D].copy()
    g = h[..., D:].copy()
    z = jnp.tanh(f) * _sigmoid(g)
    return z @ w_o
```

```python
import jax
import jax.numpy as jnp
import jax.experimental.pallas as pl
import jax.experimental.pallas.tpu as pltpu

ecs = 400

def kernel(x_ref, w_ref, wo_ref, o_ref, u_ref, acc_ref, z_ref, p_ref, os_ref):
    T, D = x_ref.shape[1], x_ref.shape[2]
    K, _, D2 = w_ref.shape
    dil = 2
    NC = D // 128
    TU = T // 2
    NS = 8
    S = TU // NS
    P = 32
    b = pl.program_id(0)

    @pl.when(b == 0)
    def _():
        for c in range(NC):
            u_ref[c, 0:P, :] = jnp.zeros((P, 128), jnp.uint32)

    for c in range(NC):
        u_ref[c, P:P + TU, :] = pltpu.bitcast(x_ref[0, :, 128 * c:128 * (c + 1)], jnp.uint32)

    def lhs_for(i):
        cols = []
        for c in range(NC):
            rows = [u_ref[c, pl.ds(P + j - i, NS, stride=S), :] for j in range(S)]
            cols.append(jnp.concatenate(rows, axis=0))
        return pltpu.bitcast(jnp.concatenate(cols, axis=1), jnp.bfloat16)

    acc_ref[...] = jnp.dot(lhs_for(0), w_ref[0], preferred_element_type=jnp.float32)
    def body(i, carry):
        acc_ref[...] += jnp.dot(lhs_for(i), w_ref[i], preferred_element_type=jnp.float32)
        return carry
    jax.lax.fori_loop(1, K, body, 0)

    def ebody(r, carry):
        rs = pl.multiple_of(r * ecs, ecs)
        h = acc_ref[pl.ds(rs, ecs), :]
        z = jnp.tanh(h[:, :D]) * jax.nn.sigmoid(h[:, D:])
        z_ref[pl.ds(rs, ecs), :] = z.astype(z_ref.dtype)
        return carry
    jax.lax.fori_loop(0, T // ecs, ebody, 0)

    o = jnp.dot(z_ref[...], wo_ref[...], preferred_element_type=jnp.float32)
    p_ref[...] = pltpu.bitcast(o.astype(jnp.bfloat16), jnp.uint32)

    for c in range(NC):
        def ubody(j, carry):
            os_ref[c, pl.ds(j, NS, stride=S), :] = p_ref[pl.ds(pl.multiple_of(NS * j, NS), NS), 128 * c:128 * (c + 1)]
            return carry
        jax.lax.fori_loop(0, S, ubody, 0)
    o_ref[0] = pltpu.bitcast(jnp.concatenate([os_ref[c] for c in range(NC)], axis=1), jnp.bfloat16)


@jax.jit
def pallas_standalone__autoregressive_conv_wavenet__speech_kernel(
    x: jax.Array,
    w: jax.Array,
    w_o: jax.Array,
):
    B, T, D = x.shape
    K = w.shape[0]
    TU = T // 2
    return pl.pallas_call(
        kernel,
        grid=(B,),
        in_specs=[
            pl.BlockSpec((1, T, D), lambda b: (b, 0, 0)),
            pl.BlockSpec((K, D, 2 * D), lambda b: (0, 0, 0), pipeline_mode=pl.Buffered(1)),
            pl.BlockSpec((D, D), lambda b: (0, 0), pipeline_mode=pl.Buffered(1)),
        ],
        out_specs=pl.BlockSpec((1, T, D), lambda b: (b, 0, 0)),
        out_shape=jax.ShapeDtypeStruct((B, T, D), x.dtype),
        scratch_shapes=[
            pltpu.VMEM((D // 128, TU + 32, 128), jnp.uint32),
            pltpu.VMEM((T, 2 * D), jnp.float32),
            pltpu.VMEM((T, D), jnp.bfloat16),
            pltpu.VMEM((TU, D), jnp.uint32),
            pltpu.VMEM((D // 128, TU, 128), jnp.uint32),
        ],
        compiler_params=pltpu.CompilerParams(
            dimension_semantics=("arbitrary",), vmem_limit_bytes=120 * 1024 * 1024),
    )(x, w, w_o)
```

```python
import jax, jax.numpy as jnp
import jax.experimental.pallas as pl
import jax.experimental.pallas.tpu as pltpu

NS = 8
P = 32
NOC = 4
PF = 64

def kernel(x_hbm, w_hbm, wo_hbm, out_hbm, u_ref, w_ref, wo_ref, acc_ref, z_ref, pz_ref, ob_ref,
           xsem, wsem, osem):
    B, T, D = x_hbm.shape
    K, _, D2 = w_hbm.shape
    NC = D // 128
    TU = T // 2
    S = TU // NS
    b = pl.program_id(0)
    nb = pl.num_programs(0)
    xu_hbm = x_hbm.bitcast(jnp.uint32)

    def x_copy(bb, slot, c):
        return pltpu.make_async_copy(
            xu_hbm.at[bb, :, pl.ds(128 * c, 128)],
            u_ref.at[slot, c, pl.ds(P, TU), :],
            xsem.at[slot, c])

    def w_copy(i):
        return pltpu.make_async_copy(w_hbm.at[i], w_ref.at[i], wsem.at[i])

    def wo_copy():
        return pltpu.make_async_copy(wo_hbm, wo_ref, wsem.at[K])

    RC = T // NOC
    def o_copy(bb, slot, r):
        return pltpu.make_async_copy(
            ob_ref.at[slot, pl.ds(r * RC, RC), :],
            out_hbm.at[bb, pl.ds(r * RC, RC), :],
            osem.at[slot, r])

    @pl.when(b == 0)
    def _():
        for c in range(NC):
            x_copy(0, 0, c).start()
        w_copy(0).start()
        for slot in range(2):
            for c in range(NC):
                u_ref[slot, c, 0:P, :] = jnp.zeros((P, 128), u_ref.dtype)
        for c in range(NC):
            pz_ref[c, 0:PF, :] = jnp.zeros((PF, 128), pz_ref.dtype)
            pz_ref[c, PF + TU:, :] = jnp.zeros((pz_ref.shape[1] - PF - TU, 128), pz_ref.dtype)

    slot = b % 2
    for c in range(NC):
        x_copy(b, slot, c).wait()

    @pl.when(b == 0)
    def _():
        for i in range(1, K):
            w_copy(i).start()
        wo_copy().start()

    @pl.when(b + 1 < nb)
    def _():
        for c in range(NC):
            x_copy(b + 1, 1 - slot, c).start()

    def lhs_for(i):
        cols = []
        for c in range(NC):
            rows = [u_ref[slot, c, pl.ds(P + j - i, NS, stride=S), :] for j in range(S)]
            cols.append(jnp.concatenate(rows, axis=0))
        return pltpu.bitcast(jnp.concatenate(cols, axis=1), jnp.bfloat16)

    def wait_w(i):
        @pl.when(b == 0)
        def _():
            w_copy(i).wait()

    wait_w(0)
    acc_ref[...] = jnp.dot(lhs_for(0), w_ref[0], preferred_element_type=jnp.float32)
    def body(i, carry):
        wait_w(i)
        acc_ref[...] += jnp.dot(lhs_for(i), w_ref[i], preferred_element_type=jnp.float32)
        return carry
    jax.lax.fori_loop(1, K - 1, body, 0)
    wait_w(K - 1)
    h = acc_ref[...] + jnp.dot(lhs_for(K - 1), w_ref[K - 1], preferred_element_type=jnp.float32)
    z = jnp.tanh(h[:, :D]) * jax.nn.sigmoid(h[:, D:])
    zu = pltpu.bitcast(z.astype(jnp.bfloat16), jnp.uint32)
    for c in range(NC):
        pz_ref[c, PF:PF + TU, :] = zu[:, 128 * c:128 * (c + 1)]

    sub = jax.lax.broadcasted_iota(jnp.int32, (NS, 128), 0)
    def natural_vreg(m, c):
        sg = (NS * m) // S
        s0 = S * (sg + 1) - NS * m
        def rows(seg):
            base = PF + NS * NS * m - (TU - 1) * seg
            assert 0 <= base and base + NS * (NS - 1) < pz_ref.shape[1]
            return pz_ref[c, pl.ds(base, NS, stride=NS), :]
        va = rows(sg)
        if s0 >= NS:
            return va
        vb = rows(sg + 1)
        return jnp.where(sub < s0, va, vb)
    for m in range(TU // NS):
        row = jnp.concatenate([natural_vreg(m, c) for c in range(NC)], axis=1)
        z_ref[2 * NS * m:2 * NS * (m + 1), :] = pltpu.bitcast(row, jnp.bfloat16)

    @pl.when(b == 0)
    def _():
        wo_copy().wait()

    @pl.when(b >= 2)
    def _():
        for r in range(NOC):
            o_copy(b - 2, slot, r).wait()

    for r in range(NOC):
        o = jnp.dot(z_ref[r * RC:(r + 1) * RC, :], wo_ref[...], preferred_element_type=jnp.float32)
        ob_ref[slot, r * RC:(r + 1) * RC, :] = o.astype(ob_ref.dtype)
        o_copy(b, slot, r).start()

    @pl.when(b == nb - 1)
    def _():
        for bb in range(2):
            @pl.when(b - bb >= 0)
            def _():
                for r in range(NOC):
                    o_copy(b - bb, (b - bb) % 2, r).wait()


@jax.jit
def pallas_standalone__autoregressive_conv_wavenet__speech_kernel(
    x: jax.Array,
    w: jax.Array,
    w_o: jax.Array,
):
    B, T, D = x.shape
    K = w.shape[0]
    TU = T // 2
    NC = D // 128
    return pl.pallas_call(
        kernel,
        grid=(B,),
        in_specs=[pl.BlockSpec(memory_space=pl.ANY)] * 3,
        out_specs=pl.BlockSpec(memory_space=pl.ANY),
        out_shape=jax.ShapeDtypeStruct((B, T, D), x.dtype),
        scratch_shapes=[
            pltpu.VMEM((2, NC, TU + P, 128), jnp.uint32),
            pltpu.VMEM((K, D, 2 * D), w.dtype),
            pltpu.VMEM((D, D), w_o.dtype),
            pltpu.VMEM((T, 2 * D), jnp.float32),
            pltpu.VMEM((T, D), jnp.bfloat16),
            pltpu.VMEM((NC, TU + 2 * PF, 128), jnp.uint32),
            pltpu.VMEM((2, T, D), x.dtype),
            pltpu.SemaphoreType.DMA((2, NC)),
            pltpu.SemaphoreType.DMA((K + 1,)),
            pltpu.SemaphoreType.DMA((2, NOC)),
        ],
        compiler_params=pltpu.CompilerParams(dimension_semantics=("arbitrary",), vmem_limit_bytes=120 * 1024 * 1024),
    )(x, w, w_o)
```

```python
import jax
import jax.numpy as jnp
import jax.experimental.pallas as pl
import jax.experimental.pallas.tpu as pltpu

NS = 8
P = 32
NOC = 4
PF = 64

def _kernel(x_hbm, w_hbm, wo_hbm, out_hbm, u_ref, w_ref, wo_ref, acc_ref, z_ref, pz_ref, ob_ref,
           xsem, wsem, osem):
    B, T, D = x_hbm.shape
    K, _, D2 = w_hbm.shape
    NC = D // 128
    TU = T // 2
    S = TU // NS
    b = pl.program_id(0)
    nb = pl.num_programs(0)
    xu_hbm = x_hbm.bitcast(jnp.uint32)

    def x_copy(bb, slot, c):
        return pltpu.make_async_copy(
            xu_hbm.at[bb, :, pl.ds(128 * c, 128)],
            u_ref.at[slot, c, pl.ds(P, TU), :],
            xsem.at[slot, c])

    def w_copy(i):
        return pltpu.make_async_copy(w_hbm.at[i], w_ref.at[i], wsem.at[i])

    def wo_copy():
        return pltpu.make_async_copy(wo_hbm, wo_ref, wsem.at[K])

    RC = T // NOC
    def o_copy(bb, slot, r):
        return pltpu.make_async_copy(
            ob_ref.at[slot, pl.ds(r * RC, RC), :],
            out_hbm.at[bb, pl.ds(r * RC, RC), :],
            osem.at[slot, r])

    @pl.when(b == 0)
    def _():
        for c in range(NC):
            x_copy(0, 0, c).start()
        w_copy(0).start()
        for slot in range(2):
            for c in range(NC):
                u_ref[slot, c, 0:P, :] = jnp.zeros((P, 128), u_ref.dtype)
        for c in range(NC):
            pz_ref[c, 0:PF, :] = jnp.zeros((PF, 128), pz_ref.dtype)
            pz_ref[c, PF + TU:, :] = jnp.zeros((pz_ref.shape[1] - PF - TU, 128), pz_ref.dtype)

    slot = b % 2
    for c in range(NC):
        x_copy(b, slot, c).wait()

    @pl.when(b == 0)
    def _():
        for i in range(1, K):
            w_copy(i).start()
        wo_copy().start()

    @pl.when(b + 1 < nb)
    def _():
        for c in range(NC):
            x_copy(b + 1, 1 - slot, c).start()

    def lhs_for(i):
        cols = []
        for c in range(NC):
            rows = [u_ref[slot, c, pl.ds(P + j - i, NS, stride=S), :] for j in range(S)]
            cols.append(jnp.concatenate(rows, axis=0))
        return pltpu.bitcast(jnp.concatenate(cols, axis=1), jnp.bfloat16)

    def wait_w(i):
        @pl.when(b == 0)
        def _():
            w_copy(i).wait()

    wait_w(0)
    acc_ref[...] = jnp.dot(lhs_for(0), w_ref[0], preferred_element_type=jnp.float32)
    def body(i, carry):
        wait_w(i)
        acc_ref[...] += jnp.dot(lhs_for(i), w_ref[i], preferred_element_type=jnp.float32)
        return carry
    jax.lax.fori_loop(1, K - 1, body, 0)
    wait_w(K - 1)
    h = acc_ref[...] + jnp.dot(lhs_for(K - 1), w_ref[K - 1], preferred_element_type=jnp.float32)
    z = jnp.tanh(h[:, :D]) * jax.nn.sigmoid(h[:, D:])
    zu = pltpu.bitcast(z.astype(jnp.bfloat16), jnp.uint32)
    for c in range(NC):
        pz_ref[c, PF:PF + TU, :] = zu[:, 128 * c:128 * (c + 1)]

    sub = jax.lax.broadcasted_iota(jnp.int32, (NS, 128), 0)
    def natural_vreg(m, c):
        sg = (NS * m) // S
        s0 = S * (sg + 1) - NS * m
        def rows(seg):
            base = PF + NS * NS * m - (TU - 1) * seg
            assert 0 <= base and base + NS * (NS - 1) < pz_ref.shape[1]
            return pz_ref[c, pl.ds(base, NS, stride=NS), :]
        va = rows(sg)
        if s0 >= NS:
            return va
        vb = rows(sg + 1)
        return jnp.where(sub < s0, va, vb)
    for m in range(TU // NS):
        row = jnp.concatenate([natural_vreg(m, c) for c in range(NC)], axis=1)
        z_ref[2 * NS * m:2 * NS * (m + 1), :] = pltpu.bitcast(row, jnp.bfloat16)

    @pl.when(b == 0)
    def _():
        wo_copy().wait()

    @pl.when(b >= 2)
    def _():
        for r in range(NOC):
            o_copy(b - 2, slot, r).wait()

    for r in range(NOC):
        o = jnp.dot(z_ref[r * RC:(r + 1) * RC, :], wo_ref[...], preferred_element_type=jnp.float32)
        ob_ref[slot, r * RC:(r + 1) * RC, :] = o.astype(ob_ref.dtype)
        o_copy(b, slot, r).start()

    @pl.when(b == nb - 1)
    def _():
        for bb in range(2):
            @pl.when(b - bb >= 0)
            def _():
                for r in range(NOC):
                    o_copy(b - bb, (b - bb) % 2, r).wait()


@jax.jit
def pallas_standalone__autoregressive_conv_wavenet__speech_kernel(
    x: jax.Array,
    w: jax.Array,
    w_o: jax.Array,
):
    B, T, D = x.shape
    K = w.shape[0]
    TU = T // 2
    NC = D // 128
    return pl.pallas_call(
        _kernel,
        grid=(B,),
        in_specs=[pl.BlockSpec(memory_space=pl.ANY)] * 3,
        out_specs=pl.BlockSpec(memory_space=pl.ANY),
        out_shape=jax.ShapeDtypeStruct((B, T, D), x.dtype),
        scratch_shapes=[
            pltpu.VMEM((2, NC, TU + P, 128), jnp.uint32),
            pltpu.VMEM((K, D, 2 * D), w.dtype),
            pltpu.VMEM((D, D), w_o.dtype),
            pltpu.VMEM((T, 2 * D), jnp.float32),
            pltpu.VMEM((T, D), jnp.bfloat16),
            pltpu.VMEM((NC, TU + 2 * PF, 128), jnp.uint32),
            pltpu.VMEM((2, T, D), x.dtype),
            pltpu.SemaphoreType.DMA((2, NC)),
            pltpu.SemaphoreType.DMA((K + 1,)),
            pltpu.SemaphoreType.DMA((2, NOC)),
        ],
        compiler_params=pltpu.CompilerParams(dimension_semantics=("arbitrary",), vmem_limit_bytes=120 * 1024 * 1024),
    )(x, w, w_o)
```
